```python
import os as _os
_os.environ.setdefault("JAX_PLATFORMS", "cpu")
import jax
import jax.numpy as jnp

def _softmax(x, axis=-1):
    return jax.nn.softmax(x, axis=axis)
def _gelu(x):
    return jax.nn.gelu(x, approximate=True)
def _silu(x):
    return jax.nn.silu(x)
def _sigmoid(x):
    return jax.nn.sigmoid(x)
def _layernorm(x, axis=-1, eps=1e-5):
    m = jnp.mean(x, axis=axis, keepdims=True)
    v = jnp.var(x, axis=axis, keepdims=True)
    return (x - m) / jnp.sqrt(v + eps)
def _scatter_add(tgt, idx, src, axis=0):
    return tgt.at[idx].add(src)
def _segment_sum(src, seg, n):
    return jax.ops.segment_sum(src, seg, n)
class _Rng:
    def __init__(self, key):
        self._k = key
    def _next(self):
        self._k, sub = jax.random.split(self._k)
        return sub
    def normal(self, shape):
        return jax.random.normal(self._next(), shape, dtype=jnp.bfloat16)
    def randint(self, lo, hi, shape):
        return jax.random.randint(self._next(), shape, lo, hi, dtype=jnp.int32)
    def uniform(self, shape, lo=0.0, hi=1.0):
        return jax.random.uniform(self._next(), shape, jnp.bfloat16, lo, hi)
    def permutation(self, n):
        return jax.random.permutation(self._next(), n)


kernel_name = 'parallel_sum__ssm_conv_s4__mixer_channel_mlp__prompt'

def setup_inputs():
    _rng = _Rng(jax.random.key(int.from_bytes(__import__("os").urandom(4), "little")))
    _w = (lambda a: (lambda t: t.astype(jnp.bfloat16) if jnp.issubdtype(t.dtype, jnp.floating) else t)(jnp.asarray(a)))
    def _A_setup():
        B, L, D, N = 1, 2048, 512, 128
        A_re = -jnp.exp((lambda *s: _rng.normal(s) * 0.1)(D, N))
        A_im = jnp.pi * (lambda *s: _rng.normal(s) * 0.1)(D, N)
        B_re = (lambda *s: _rng.normal(s) * 0.1)(D, N)
        B_im = (lambda *s: _rng.normal(s) * 0.1)(D, N)
        C_re = (lambda *s: _rng.normal(s) * 0.1)(D, N)
        C_im = (lambda *s: _rng.normal(s) * 0.1)(D, N)
        log_dt = (lambda *s: _rng.normal(s) * 0.1)(D) * 0.5 - 4.0
        Dskip = (lambda *s: _rng.normal(s) * 0.05)(D)
        return {
            "u": _w((lambda *s: _rng.normal(s) * 0.05)(B, L, D)),
            "A_re": _w(A_re),
            "A_im": _w(A_im),
            "B_re": _w(B_re),
            "B_im": _w(B_im),
            "C_re": _w(C_re),
            "C_im": _w(C_im),
            "log_dt": _w(log_dt),
            "Dskip": _w(Dskip),
        }
    _A_in = _A_setup()

    def _B_setup():
        B, S, D, F = 1, 2048, 512, 1792
        return {
            "x": _w((lambda *s: _rng.normal(s) * 0.05)(B, S, D)),
            "w1": _w((lambda *s: _rng.normal(s) * 0.2)(D, F) * (D ** -0.5)),
            "b1": _w((lambda *s: _rng.normal(s) * 0.2)(F)),
            "w2": _w((lambda *s: _rng.normal(s) * 0.2)(F, D) * (F ** -0.5)),
            "b2": _w((lambda *s: _rng.normal(s) * 0.05)(D)),
        }
    _B_in = _B_setup()

    return {
        "A_u": _A_in["u"],
        "A_A_re": _A_in["A_re"],
        "A_A_im": _A_in["A_im"],
        "A_B_re": _A_in["B_re"],
        "A_B_im": _A_in["B_im"],
        "A_C_re": _A_in["C_re"],
        "A_C_im": _A_in["C_im"],
        "A_log_dt": _A_in["log_dt"],
        "A_Dskip": _A_in["Dskip"],
        "B_x": _B_in["x"],
        "B_w1": _B_in["w1"],
        "B_b1": _B_in["b1"],
        "B_w2": _B_in["w2"],
        "B_b2": _B_in["b2"],
    }

def reference(A_u, A_A_re, A_A_im, A_B_re, A_B_im, A_C_re, A_C_im, A_log_dt, A_Dskip, B_x, B_w1, B_b1, B_w2, B_b2):
    def _A_ref(u, A_re, A_im, B_re, B_im, C_re, C_im, log_dt, Dskip):
        Bsz, L, D = u.shape
        dt = jnp.exp(log_dt)[:, None]
        A = A_re + 1j * A_im
        Bc = B_re + 1j * B_im
        Cc = C_re + 1j * C_im
        logdA = dt * A
        dB = dt * Bc
        l = (lambda x, dt: x.astype(dt))(jnp.arange(L), A_re.dtype)
        P = jnp.exp(logdA[:, :, None] * l[None, None, :])
        K = jnp.einsum("dn,dnl,dn->dl", Cc, P, dB).real
        L2 = 2 * L
        Kp = jnp.pad(K, ((0, 0), (0, L)))
        up = (lambda x, *d: x.transpose(*d))(u, 0, 2, 1)
        up = jnp.pad(up, ((0, 0), (0, 0), (0, L)))
        Kf = (lambda x, axes=(-2,-1): jnp.fft.rfft2(x.astype(jnp.float32), axes=axes))(Kp[:, None, :], axes=(-2, -1))
        Uf = (lambda x, axes=(-2,-1): jnp.fft.rfft2(x.astype(jnp.float32), axes=axes))(up[:, :, None, :], axes=(-2, -1))
        Yf = Uf * Kf[None, :, :, :]
        y = (lambda x, s, axes=(-2,-1): jnp.fft.irfft2(x, s=s, axes=axes).astype(jnp.bfloat16))(Yf, (1, L2), axes=(-2, -1))[:, :, 0, :L]
        y = (lambda x, *d: x.transpose(*d))(y, 0, 2, 1) + u * Dskip[None, None, :]
        return y

    def _B_ref(x, w1, b1, w2, b2):
        y = _layernorm(x, axis=-1)
        h = _gelu(jnp.einsum("bsd,df->bsf", y, w1) + b1)
        return jnp.einsum("bsf,fd->bsd", h, w2) + b2

    x = A_u
    xn = _layernorm(x, axis=-1)
    return x + _A_ref(xn, A_A_re, A_A_im, A_B_re, A_B_im, A_C_re, A_C_im, A_log_dt, A_Dskip) + _B_ref(xn, B_w1, B_b1, B_w2, B_b2)
```

```python
import functools

import numpy as np
import jax
import jax.numpy as jnp
import jax.experimental.pallas as pl
import jax.experimental.pallas.tpu as pltpu

L, D, N, F = 2048, 512, 128, 1792
Q = 128
NB = L // Q
NG = D // 128
BS = 136
PS = NB * BS + 8
VS = 136
S = 132
F32, BF16, I32 = jnp.float32, jnp.bfloat16, jnp.int32


def _np_bf16_bits(a):
    u = np.ascontiguousarray(a, dtype=np.float32).view(np.uint32).astype(np.uint64)
    r = (u + 0x7FFF + ((u >> 16) & 1)) >> 16
    return r.astype(np.uint32)


def _np_bf16_round(a):
    return (_np_bf16_bits(a) << 16).view(np.float32)


def _np_pack_rows(a):
    b = _np_bf16_bits(a)
    return (b[0::2] | (b[1::2] << 16)).view(np.int32)


def _bpos(b):
    j, t, r = b // 16, (b % 16) // 8, b % 8
    return 16 * j + 2 * r + t


def _make_consts():
    lb = _np_bf16_round(np.arange(L, dtype=np.float32)).astype(np.int64)
    k = np.concatenate([np.arange(0, Q, 2), np.arange(1, Q, 2)]).astype(np.float64)
    l = np.arange(Q, dtype=np.float64)
    th = 2.0 * np.pi * (k[:, None] + 0.5) * l[None, :] / (2 * Q)
    fm = np.concatenate([np.cos(th), -np.sin(th)], 0)
    mats, cls = [fm], []
    for i in range(NB):
        m = np.zeros((2 * Q, Q))
        for ll in range(Q):
            b = int(lb[Q * i + ll]) - Q * i
            assert 0 <= b <= Q
            if b == Q:
                assert i >= 2
                b = 1
            else:
                assert i < 2 or b != 1
            m[:, _bpos(b)] += fm[:, ll]
        for c, mm in enumerate(mats):
            if c > 0 and np.array_equal(mm, m):
                cls.append(c)
                break
        else:
            mats.append(m)
            cls.append(len(mats) - 1)
    thi = 2.0 * np.pi * (k[None, :] + 0.5) * l[:, None] / (2 * Q)
    gr, gi = np.cos(thi) / Q, -np.sin(thi) / Q
    g = np.stack([gr, gi], 2).reshape(Q, 2 * Q)
    mc = np.stack([_np_pack_rows(m) for m in mats])
    gp = np.stack([_np_pack_rows(g[:, :Q]), _np_pack_rows(g[:, Q:])])
    return mc, gp, tuple(cls)


_MC, _GP, _CLS = _make_consts()
_ABSENT = 0x7FC17FC1
assert not (_MC == _ABSENT).any()


def _cmul(ar, ai, br, bi):
    return ar * br - ai * bi, ar * bi + ai * br


def _csq(ar, ai):
    t = ar * ai
    return ar * ar - ai * ai, t + t


def _nt(a, b):
    return jax.lax.dot_general(a, b, (((1,), (1,)), ((), ())), preferred_element_type=F32)


def _nn(a, b):
    return jnp.dot(a, b, preferred_element_type=F32)


def _pack(lo, hi):
    return pltpu.pack_elementwise([lo, hi], packed_dtype=BF16)


def _unpack(w):
    return (pltpu.unpack_elementwise(w, index=0, packed_dtype=BF16, unpacked_dtype=F32),
            pltpu.unpack_elementwise(w, index=1, packed_dtype=BF16, unpacked_dtype=F32))


def _bf(w):
    return pltpu.bitcast(w, BF16)


def _gelu(x):
    c1 = 0.7978845608028654
    c2 = 0.7978845608028654 * 0.044715
    inner = x * (c1 + c2 * (x * x))
    hx = 0.5 * x
    return hx + hx * jnp.tanh(inner)


def interleave(*streams):
    state = [[g, 0.0, float(w)] for g, w in streams if w > 0]
    while state:
        st = min(state, key=lambda s: s[1] / s[2])
        try:
            st[1] += next(st[0])
        except StopIteration:
            state.remove(st)


def interleave2(*streams):
    state = [[g, 0.0, float(w), a, b] for g, w, a, b in streams if w > 0]
    tm = lambda s: s[3] + (s[4] - s[3]) * s[1] / s[2]
    lead = state[0]
    while state:
        st = min(state, key=tm)
        if st is lead:
            CLOCK[0] = tm(st)
            CLOCK[2] = (lead[4] - lead[3]) / lead[2]
        CLOCK[1] = tm(st)
        try:
            st[1] += next(st[0])
        except StopIteration:
            state.remove(st)


CLOCK = [0.0, 0.0, 1.0]


def run(gen):
    for _ in gen:
        pass


def chain(*gens):
    for g in gens:
        yield from g


class K:
    NAMES = ("x_hbm w1_hbm w2_hbm are aim bre bim cre cim ldt dsk b1 b2 mc gp out_hbm "
             "x_s w1_s w2_s xn_s dt_s vbr vbi lar lai zz xk vs ku y_s r_s acc_s h_s st_s o_s "
             "sems osems").split()

    def __init__(self, refs, cfg):
        assert len(refs) == len(self.NAMES)
        (self.x_hbm, self.w1_hbm, self.w2_hbm, self.are, self.aim, self.bre, self.bim, self.cre, self.cim, self.ldt, self.dsk, self.b1, self.b2, self.mc, self.gp, self.out_hbm, self.x_s, self.w1_s, self.w2_s, self.xn_s, self.dt_s, self.vbr, self.vbi, self.lar, self.lai, self.zz, self.xk, self.vs, self.ku, self.y_s, self.r_s, self.acc_s, self.h_s, self.st_s, self.o_s, self.sems, self.osems) = refs
        self.cfg = cfg
        self.MT, self.FC, self.MB = cfg["MT"], cfg["FC"], cfg["MB"]

    @staticmethod
    def scratch(cfg):
        MT = cfg["MT"]
        return [
            pltpu.VMEM((L // 2, D), I32), pltpu.VMEM((D // 2, F), I32), pltpu.VMEM((F // 2, D), I32),
            pltpu.VMEM((NG, L // 2, 128), I32),
            pltpu.VMEM((D, 128), F32),
            pltpu.VMEM((8 * S, 128), F32), pltpu.VMEM((8 * S, 128), F32),
            pltpu.VMEM((NB * S, 128), F32), pltpu.VMEM((NB * S, 128), F32),
            pltpu.VMEM((8 * 128, 128), F32),
            pltpu.VMEM(((NB + 1) * S, 128), F32),
            pltpu.VMEM((128 * VS + 8 * 128 + 8, 128), I32),
            pltpu.VMEM((6 * PS, 128), F32),
            pltpu.VMEM((NB, 128, 128), I32),
            pltpu.VMEM((NG, L, 128), F32),
            pltpu.VMEM((L, D), F32),
            pltpu.VMEM((F // 128, MT, 128), BF16),
            pltpu.VMEM((4, L // 2, 128), F32),
            pltpu.VMEM((L, D), BF16),
            pltpu.SemaphoreType.DMA((3,)),
            pltpu.SemaphoreType.DMA((L // MT,)),
        ]

    @staticmethod
    def rows(g, n=128):
        if isinstance(g, int):
            return pl.ds(g * n, n)
        return pl.ds(pl.multiple_of(g * n, 8), n)

    tokens = None

    def post(self, v, weight=1.0):
        self.tokens = [v[r:r + 8, 0:128] for r in range(0, v.shape[0], 16)]
        self.tok_w = weight

    def tie(self, *vs):
        if self.tokens is None or not self.cfg.get("tie", True):
            return vs
        frac = (CLOCK[1] - CLOCK[0]) / (CLOCK[2] * self.tok_w)
        tok = self.tokens[max(0, min(len(self.tokens) - 1, int(frac * len(self.tokens))))]
        m = self.mc[0, 0:8, :] != _ABSENT
        out = []
        for v in vs:
            if v.ndim == 2 and v.shape != (8, 128):
                n = v.shape[0] // 8
                out.append(jnp.where(m[None], v.reshape(n, 8, 128), tok[None]).reshape(v.shape))
            else:
                out.append(jnp.where(m, v, tok))
        return out

    def dt_phase(self):
        dt_row = jnp.exp(self.ldt[...].astype(F32)).astype(BF16).astype(F32)
        for g in range(NG):
            self.dt_s[pl.ds(g * 128, 128), :] = jnp.broadcast_to(dt_row[g:g + 1, :], (128, 128)).T
            yield 1

    kv_done = 0
    id_done = 0
    kd_done = 128
    mac_running = False
    p_done = False
    du_done = 0
    mac_done = True

    def precompute(self, g):
        assert self.kd_done == 128 or self.cfg.get("mode", "full") != "full"
        self.p_done = False
        self.kv_done = 0
        self.kd_done = 0
        PC = self.cfg.get("PC", 32)
        self.p_rows = 0
        for c in range(128 // PC):
            if isinstance(g, int):
                src = pl.ds(g * 128 + c * PC, PC)
            else:
                src = pl.ds(pl.multiple_of(g * 128 + c * PC, 8), PC)
            dt, = self.tie(self.dt_s[src, :])
            ld = lambda ref: ref[src, :].astype(F32)
            lr = dt * ld(self.are)
            li = dt * ld(self.aim)
            br = dt * ld(self.bre)
            bi = dt * ld(self.bim)
            cr, ci = ld(self.cre), ld(self.cim)
            a = (cr * br - ci * bi, -(cr * bi + ci * br))
            mag = jnp.exp(lr)
            z1 = (mag * jnp.cos(li), mag * jnp.sin(li))
            yield 3 * PC / 32
            z2 = _csq(*z1)
            z3 = _cmul(*z2, *z1)
            z4 = _csq(*z2)
            z5 = _cmul(*z4, *z1)
            z6 = _csq(*z3)
            z7 = _cmul(*z4, *z3)
            pw = [(jnp.ones((PC, 128), F32), jnp.zeros((PC, 128), F32)), z1, z2, z3, z4, z5, z6, z7]
            for b0 in range(8):
                self.vbr[pl.ds(b0 * S + c * PC, PC), :] = pw[b0][0]
                self.vbi[pl.ds(b0 * S + c * PC, PC), :] = pw[b0][1]
            z8 = _csq(*z4)
            z16 = _csq(*z8)
            z32 = _csq(*z16)
            z64 = _csq(*z32)
            z128 = _csq(*z64)
            for q, z in enumerate((z8, z16, z32, z64)):
                self.zz[pl.ds((2 * q) * 128 + c * PC, PC), :] = z[0]
                self.zz[pl.ds((2 * q + 1) * 128 + c * PC, PC), :] = z[1]
            yield 2 * PC / 32
            zc = (z128[0], -z128[1])
            for i in range(NB):
                slab = (i // 2) + 8 * (i % 2)
                self.lar[pl.ds(slab * S + c * PC, PC), :] = a[0]
                self.lai[pl.ds(slab * S + c * PC, PC), :] = a[1]
                a = _cmul(*a, *zc)
                if i % 8 == 7:
                    yield 1.5 * PC / 32
            k2048 = jnp.sum(a[0], axis=1, keepdims=True)
            self.xk[pl.ds(NB * S + c * PC, PC), :] = jnp.broadcast_to(k2048, (PC, 128))
            self.p_rows = (c + 1) * PC

    def kgen(self):
        for d in range(128):
            vr = self.vbr[pl.ds(d, 8, stride=S), :][None]
            vi = self.vbi[pl.ds(d, 8, stride=S), :][None]
            for q in range(4):
                zr = jnp.broadcast_to(self.zz[pl.ds((2 * q) * 128 + d, 1), :], (8, 128))[None]
                zi = jnp.broadcast_to(self.zz[pl.ds((2 * q + 1) * 128 + d, 1), :], (8, 128))[None]
                nr, ni = _cmul(vr, vi, zr, zi)
                vr = jnp.concatenate([vr, nr], axis=0)
                vi = jnp.concatenate([vi, ni], axis=0)
            pk = lambda v: _bf(jnp.concatenate([_pack(v[2 * j], v[2 * j + 1]) for j in range(8)], axis=0))
            lk = lambda ref: _bf(_pack(ref[pl.ds(d, 8, stride=S), :], ref[pl.ds(8 * S + d, 8, stride=S), :]))
            o = _nt(lk(self.lar), pk(vr)) + _nt(lk(self.lai), pk(vi))
            self.xk[pl.ds(d, NB, stride=S), :] = o
            yield 1

    def kgen_v(self, g=None):
        for d in range(128):
            assert self.p_rows > d or self.cfg.get("mode", "full") != "full", "KV emitted before P"

            def zb(q, tie):
                zr = jnp.broadcast_to(self.zz[pl.ds((2 * q) * 128 + d, 1), :], (8, 128))
                zi = jnp.broadcast_to(self.zz[pl.ds((2 * q + 1) * 128 + d, 1), :], (8, 128))
                return self.tie(zr, zi) if tie else (zr, zi)

            def put(j, a, b):
                self.vs[pl.ds(d * VS + 8 * j, 8), :] = _pack(a[0], b[0])
                self.vs[pl.ds(d * VS + 64 + 8 * j, 8), :] = _pack(a[1], b[1])
            v = [(self.vbr[pl.ds(d, 8, stride=S), :], self.vbi[pl.ds(d, 8, stride=S), :])]
            z = zb(0, True)
            v.append(_cmul(*v[0], *z))
            z = zb(1, False)
            v += [_cmul(*v[0], *z), _cmul(*v[1], *z)]
            put(0, v[0], v[1])
            put(1, v[2], v[3])
            yield 0.22
            z = zb(2, True)
            v += [_cmul(*v[j], *z) for j in range(4)]
            put(2, v[4], v[5])
            put(3, v[6], v[7])
            yield 0.26
            z = zb(3, True)
            w = [_cmul(*v[j], *z) for j in range(4)]
            put(4, w[0], w[1])
            put(5, w[2], w[3])
            yield 0.26
            z = self.tie(*z)
            w = [_cmul(*v[j], *z) for j in range(4, 8)]
            put(6, w[0], w[1])
            put(7, w[2], w[3])
            self.kv_done = d + 1
            yield 0.26

    def kgen_d(self, g=None):
        for d in range(128):
            assert self.kv_done > d or self.cfg.get("mode", "full") != "full", "KD emitted before KV"
            lk = lambda ref: _bf(_pack(ref[pl.ds(d, 8, stride=S), :], ref[pl.ds(8 * S + d, 8, stride=S), :]))
            o = (_nt(lk(self.lar), _bf(self.vs[pl.ds(d * VS, 64), :]))
                 + _nt(lk(self.lai), _bf(self.vs[pl.ds(d * VS + 64, 64), :])))
            self.xk[pl.ds(d, NB, stride=S), :] = o
            self.kd_done = d + 1
            yield 1

    def dft_k(self):
        lane = jax.lax.broadcasted_iota(I32, (128, 128), 1)
        prev = None
        full = self.cfg.get("mode", "full") == "full"
        assert not full or (self.kd_done == 128 and not self.mac_running), "DK emitted too early"
        for i in range(NB):
            xt = self.xk[pl.ds(i * S, 128), :]
            if i >= 2:
                nx = self.xk[pl.ds((i + 1) * S, 128), :]
                xt = jnp.where(lane == _bpos(1), pltpu.roll(nx, _bpos(1), 1), xt)
            kf = _nt(_bf(self.mc[_CLS[i]]), xt.astype(BF16))
            a, b = kf[:128], kf[128:]
            if prev is None:
                c, dd = a, b
            else:
                pa, pb = prev
                c = jnp.concatenate([a[:64] - pb[:64], a[64:] + pb[64:]], axis=0)
                dd = jnp.concatenate([b[:64] + pa[:64], b[64:] - pa[64:]], axis=0)
            prev = (a, b)
            self.ku[pl.ds(0 * PS + i * BS, 128), :] = c
            self.ku[pl.ds(1 * PS + i * BS, 128), :] = dd - c
            self.ku[pl.ds(2 * PS + i * BS, 128), :] = dd + c
            yield 1

    def dft_u(self, g):
        assert self.mac_done
        self.du_done = 0
        for j in range(NB):
            uf = _nn(_bf(self.mc[0]), _bf(self.xn_s[g, pl.ds(j * 64, 64), :]))
            a, b = uf[:128], uf[128:]
            self.ku[pl.ds(3 * PS + j * BS, 128), :] = a
            self.ku[pl.ds(4 * PS + j * BS, 128), :] = b
            self.ku[pl.ds(5 * PS + j * BS, 128), :] = a + b
            self.du_done = j + 1
            yield 1

    def mac(self):
        MB = self.MB
        assert self.du_done == 16 or self.cfg.get("mode", "full") != "full", "MAC emitted before DU"
        self.mac_running = True
        self.mac_done = False
        for v in range(16):
            def ld(q, blk):
                return self.ku[pl.ds(q * PS + blk * BS + 8 * v, 8), :]
            for mg in range(NB // MB):
                ms = list(range(mg * MB, (mg + 1) * MB))
                s1, s2, s3 = {}, {}, {}
                ucache = {}
                for i in range(ms[-1] + 1):
                    c, e, f = ld(0, i), ld(1, i), ld(2, i)
                    if i % self.cfg.get("mac_tie", 100) == 0:
                        c, e, f = self.tie(c, e, f)
                    n = 0
                    for m in ms:
                        j = m - i
                        if j < 0:
                            continue
                        if j not in ucache:
                            ucache[j] = (ld(3, j), ld(4, j), ld(5, j))
                        ua, ub, ug = ucache[j]
                        if m in s1:
                            s1[m] = s1[m] + c * ug
                            s2[m] = s2[m] + e * ua
                            s3[m] = s3[m] + f * ub
                        else:
                            s1[m], s2[m], s3[m] = c * ug, e * ua, f * ub
                        n += 1
                    yield n / 136.0
                for m in ms:
                    self.y_s[m, pl.ds(8 * v, 8), :] = _pack(s1[m] - s3[m], s1[m] + s2[m])
        self.mac_running = False
        self.mac_done = True

    def idft(self, g):
        assert self.mac_done or self.cfg.get("mode", "full") != "full", "ID emitted before MAC"
        gm = jnp.concatenate([_bf(self.gp[0]), _bf(self.gp[1])], axis=1)
        for m in range(NB):
            self.r_s[g, pl.ds(m * 128, 128), :] = _nn(gm, _bf(self.y_s[m]))
            if m == NB - 1:
                self.id_done += 1
            yield 1

    def layernorm(self):
        RC = self.cfg.get("LNRC", 8)
        n = L // 2 // RC
        inv = 1.0 / D
        for r in range(n):
            ev, od = _unpack(self.x_s[pl.ds(r * RC, RC), :])
            for t, v in enumerate((ev, od)):
                self.st_s[t, pl.ds(r * RC, RC), :] = jnp.broadcast_to(
                    jnp.sum(v, axis=1, keepdims=True) * inv, (RC, 128))
            yield 0.2
        for r in range(n):
            ev, od = _unpack(self.x_s[pl.ds(r * RC, RC), :])
            for t, v in enumerate((ev, od)):
                mu = self.st_s[t, pl.ds(r * RC, RC), :]
                sq = None
                for kk in range(NG):
                    c = v[:, kk * 128:(kk + 1) * 128] - mu
                    sq = c * c if sq is None else sq + c * c
                var = jnp.sum(sq, axis=1, keepdims=True) * inv
                self.st_s[2 + t, pl.ds(r * RC, RC), :] = jnp.broadcast_to(jax.lax.rsqrt(var + 1e-5), (RC, 128))
            yield 0.5
        for r in range(n):
            ev, od = _unpack(self.x_s[pl.ds(r * RC, RC), :])
            mu = [self.st_s[t, pl.ds(r * RC, RC), :] for t in range(2)]
            rs = [self.st_s[2 + t, pl.ds(r * RC, RC), :] for t in range(2)]
            for kk in range(NG):
                sl = slice(kk * 128, (kk + 1) * 128)
                self.xn_s[kk, pl.ds(r * RC, RC), :] = _pack((ev[:, sl] - mu[0]) * rs[0], (od[:, sl] - mu[1]) * rs[1])
            yield 0.3

    def mlp(self, r, sink):
        MT, FC = self.MT, self.FC
        RS = self.cfg.get("RS", MT)
        mode = self.cfg.get("accmode", "ssa")
        nch = F // FC

        def xload(t):
            if isinstance(r, int):
                rr = pl.ds(r * (MT // 2) + t * (RS // 2), RS // 2)
            else:
                rr = pl.ds(pl.multiple_of(r * (MT // 2) + t * (RS // 2), 8), RS // 2)
            return jnp.concatenate([_bf(self.xn_s[kk, rr, :]) for kk in range(NG)], axis=1)

        def arows(t):
            if isinstance(r, int):
                return pl.ds(r * MT + t * RS, RS)
            return pl.ds(pl.multiple_of(r * MT + t * RS, 8), RS)

        xts = [xload(t) for t in range(MT // RS)] if self.cfg.get("xload", "once") == "once" else None
        acc = [None] * (MT // RS)
        if mode == "big":
            for t in range(MT // RS):
                for c in range(nch):
                    bias = jnp.concatenate(
                        [self.b1[pl.ds(c * (FC // 128) + u, 1), :] for u in range(FC // 128)], axis=1).astype(F32)
                    xt = xts[t] if xts is not None else xload(t)
                    h = _nn(xt, _bf(self.w1_s[:, c * FC:(c + 1) * FC])) + bias
                    h = _gelu(h)
                    for u in range(FC // 128):
                        hh = h[:, u * 128:(u + 1) * 128].astype(BF16)
                        self.h_s[c * (FC // 128) + u, pl.ds(t * RS, RS), :] = hh
                    yield 1 * RS / MT
            NC = self.cfg.get("NC", 512)
            outs = []
            for t in range(MT // RS):
                row = []
                for n0 in range(0, D, NC):
                    hh = jnp.concatenate([self.h_s[u, pl.ds(t * RS, RS), :] for u in range(F // 128)], axis=1)
                    row.append(_nn(hh, _bf(self.w2_s[:, n0:n0 + NC])))
                    yield nch * (RS / MT) * (NC / D)
                outs.append(jnp.concatenate(row, axis=1))
            yield from sink(r, jnp.concatenate(outs, axis=0))
            return
        for c in range(nch):
            for t in range(MT // RS):
                bias = jnp.concatenate(
                    [self.b1[pl.ds(c * (FC // 128) + u, 1), :] for u in range(FC // 128)], axis=1).astype(F32)
                xt = xts[t] if xts is not None else xload(t)
                h = _nn(xt, _bf(self.w1_s[:, c * FC:(c + 1) * FC])) + bias
                self.post(h, RS / MT)
                yield 1 * RS / MT
                h = _gelu(h).astype(BF16)
                p = _nn(h, _bf(self.w2_s[c * FC // 2:(c + 1) * FC // 2, :]))
                self.post(p, RS / MT)
                if mode == "ssa":
                    acc[t] = p if acc[t] is None else acc[t] + p
                else:
                    if c == 0:
                        self.acc_s[arows(t), :] = p
                    elif c < nch - 1 or sink == self.sink_store:
                        self.acc_s[arows(t), :] += p
                    else:
                        acc[t] = self.acc_s[arows(t), :] + p
                yield 1 * RS / MT
        if mode == "mem" and sink == self.sink_store:
            return
        yield from sink(r, jnp.concatenate(acc, axis=0))

    def sink_store(self, r, acc):
        self.acc_s[self.rows(r, self.MT), :] = acc
        yield 0.01

    def finalize(self, r, acc):
        assert acc is not None or (self.last_seen and self.id_done == self.id_need), "finalize before last ID"
        MT = self.MT
        dsk_row = jnp.concatenate([self.dsk[pl.ds(g, 1), :] for g in range(NG)], axis=1).astype(F32)
        b2_row = jnp.concatenate([self.b2[pl.ds(g, 1), :] for g in range(NG)], axis=1).astype(F32)
        RC = 64
        for t in range(MT // RC):
            r0 = r * MT + t * RC
            a = acc[t * RC:(t + 1) * RC] if acc is not None else self.acc_s[pl.ds(r0, RC), :]
            y = jnp.concatenate([self.r_s[g, pl.ds(r0, RC), :] for g in range(NG)], axis=1)
            xx = _bf(self.x_s[pl.ds(r0 // 2, RC // 2), :]).astype(F32)
            xn = jnp.concatenate(
                [_bf(self.xn_s[g, pl.ds(r0 // 2, RC // 2), :]) for g in range(NG)], axis=1).astype(F32)
            self.o_s[pl.ds(r0, RC), :] = (xx + (y + xn * dsk_row) + (a + b2_row)).astype(BF16)
            yield 0.2
        cp = pltpu.make_async_copy(self.o_s.at[pl.ds(r * MT, MT)], self.out_hbm.at[pl.ds(r * MT, MT)],
                                   self.osems.at[r])
        cp.start()
        self.cps.append(cp)

    def conv_k(self, g):
        return chain(scale(self.precompute(g), 4.0 / 32), scale(self.kgen(), 14.0 / 128), scale(self.dft_k(), 1.5 / 16))

    def conv_u(self, g):
        return chain(scale(self.dft_u(g), 1.0 / 16), scale(self.mac(), 13.0 / 16), scale(self.idft(g), 1.0 / 16))


def scale(gen, f):
    for w in gen:
        yield w * f


DBG = "acc_s xn_s dt_s vbr vbi lar lai zz xk vs ku y_s r_s".split()


def _make_kernel(cfg):
    def kernel(*refs):
        mode = cfg.get("mode", "full")
        if mode != "full":
            n_in = 15
            dbg = refs[n_in + 1:n_in + 1 + len(DBG)]
            refs = refs[:n_in + 1] + refs[n_in + 1 + len(DBG):]
        k = K(refs, cfg)
        k.dyn0 = pl.program_id(0) * 8 if cfg.get("dyn", False) else 0
        MT = k.MT
        NT_ = L // MT
        per = NT_ // NG
        k.cps = []
        if mode not in ("full", "STEP", "LAST"):
            g = pl.program_id(0) if cfg.get("dyn", False) else 1
            ph = dict(P=lambda: k.precompute(g), KG=k.kgen, KV=k.kgen_v, KD=k.kgen_d, DK=k.dft_k, DU=lambda: k.dft_u(g), MAC=k.mac,
                      ID=lambda: k.idft(g), LN=k.layernorm, DT=k.dt_phase,
                      MLP=lambda: chain(*[k.mlp(r, k.sink_store) for r in range(per)]),
                      CK=lambda: k.conv_k(g), CU=lambda: k.conv_u(g),
                      C=lambda: chain(k.conv_k(g), k.conv_u(g)),
                      FIN=lambda: k.finalize(0, None))
            tot = dict(P=32, KG=128, KV=128, KD=128, DK=16, DU=16, MAC=16, ID=16, LN=32, DT=4, MLP=per * 2 * (F // k.FC),
                       CK=19.5, CU=15, C=34.5, FIN=MT / 64 * 0.2)
            if ">" in mode:
                for n in mode.split(">"):
                    run(ph[n]())
            else:
                names = mode.split("+")
                interleave2(*[(ph[n](), tot[n], *cfg.get("t_" + n, (0.0, 1.0))) for n in names])
            for cp in k.cps:
                cp.wait()
            for n, o in zip(DBG, dbg):
                pltpu.sync_copy(getattr(k, n), o)
            return

        cp_x = pltpu.make_async_copy(k.x_hbm.bitcast(I32), k.x_s, k.sems.at[0])
        cp_w1 = pltpu.make_async_copy(k.w1_hbm.bitcast(I32), k.w1_s, k.sems.at[1])
        cp_w2 = pltpu.make_async_copy(k.w2_hbm.bitcast(I32), k.w2_s, k.sems.at[2])
        cp_x.start()
        cp_w1.start()
        cp_w2.start()
        if cfg.get("poison"):
            for n in ("vbr", "vbi", "lar", "lai", "zz", "xk", "ku", "r_s", "acc_s", "st_s", "dt_s"):
                ref = getattr(k, n)
                ref[...] = jnp.full(ref.shape, 1e4, F32)
            for n in ("vs", "y_s", "xn_s"):
                ref = getattr(k, n)
                ref[...] = jnp.full(ref.shape, 0x461C461C, I32)
        nch = F // k.FC
        mlp_w = per * 2 * nch
        only = cfg.get("only")
        T = dict(cfg["T"], **cfg.get("T2", {}))
        PW = 128 // cfg["PC"] * 6.5 * cfg["PC"] / 32

        if only == "LN":
            run(k.layernorm())
            pltpu.sync_copy(k.xn_s.at[0], k.out_hbm.at[pl.ds(0, 512), pl.ds(0, 128)].bitcast(I32).at[pl.ds(0, 1)]) if False else None
            for kk in range(NG):
                pltpu.sync_copy(k.xn_s.at[kk], k.out_hbm.bitcast(I32).at[:, pl.ds(kk * 128, 128)])
            return
        if mode == "full":
            run(k.dt_phase())
            run(k.precompute(0))
            interleave2((k.kgen_v(0), 128, 0.0, 1.0), (k.kgen_d(0), 128, 0.02, 1.02))
            run(k.dft_k())
        cp_x.wait()
        k.tokens = None
        if mode == "full":
            run(k.layernorm())
        cp_w1.wait()
        cp_w2.wait()

        def step(g, last):
            k.tokens = None
            rs = [g * per + t for t in range(per)]
            if not last:
                interleave2(
                    (chain(*[k.mlp(r, k.sink_store) for r in rs]), mlp_w, 0.0, 1.0),
                    (k.dft_u(g), 16, *T["DU"]),
                    (k.precompute(g + 1), PW, *T["P"]),
                    (k.mac(), 16, *T["MAC"]),
                    (k.kgen_v(g + 1), 128, *T["KV"]),
                    (k.kgen_d(g + 1), 128, *T["KD"]),
                    (k.idft(g), 16, *T["ID"]),
                    (k.dft_k(), 16, *T["DK"]),
                )
            else:
                k.last_seen = True
                k.id_need = k.id_done + 1
                first = [r for r in range(NT_ - 1)]
                interleave2(
                    (chain(*[k.mlp(r, k.finalize if r == NT_ - 1 else k.sink_store) for r in rs]),
                     mlp_w + MT / 64 * 0.2, 0.0, 1.0),
                    (k.dft_u(g), 16, *T["DU3"]),
                    (k.mac(), 16, *T["MAC3"]),
                    (k.idft(g), 16, *T["ID3"]),
                    (chain(*[k.finalize(r, None) for r in first]), len(first) * MT / 64 * 0.2, *T["FIN3"]),
                )

        if mode != "LAST":
            if cfg.get("use_loop", True):
                def body(g, c):
                    step(g, False)
                    return c
                jax.lax.fori_loop(0, NG - 1, body, 0)
            else:
                for g in range(NG - 1):
                    step(g, False)
        if mode != "STEP":
            step(NG - 1, True)
        for cp in k.cps:
            cp.wait()
        if mode != "full":
            for n, o in zip(DBG, dbg):
                pltpu.sync_copy(getattr(k, n), o)

    return kernel


def build(**cfg):
    cfg = dict(dict(MT=256, FC=128, MB=2, use_loop=True, vmem_mb=110, xload="perdot", accmode="mem", mac_tie=4, PC=16,
                    T=dict(DU=(0.0, 0.06), P=(0.0, 0.12), MAC=(0.07, 0.86), KV=(0.13, 0.84), KD=(0.14, 0.86),
                           ID=(0.87, 0.93), DK=(0.9, 0.99),
                           DU3=(0.0, 0.06), MAC3=(0.07, 0.55), ID3=(0.56, 0.62), FIN3=(0.63, 0.97))), **cfg)

    def fn(A_u, A_A_re, A_A_im, A_B_re, A_B_im, A_C_re, A_C_im, A_log_dt, A_Dskip, B_x, B_w1, B_b1, B_w2, B_b2):
        x = A_u.reshape(L, D)
        anyspec = pl.BlockSpec(memory_space=pl.ANY)
        vm = pl.BlockSpec(memory_space=pltpu.VMEM)
        sc = K.scratch(cfg)
        extra = []
        if cfg.get("mode", "full") != "full":
            base = K.NAMES.index("x_s")
            extra = [jax.ShapeDtypeStruct(sc[K.NAMES.index(n) - base].shape, sc[K.NAMES.index(n) - base].dtype) for n in DBG]
        out = pl.pallas_call(
            _make_kernel(cfg),
            out_shape=[jax.ShapeDtypeStruct((L, D), BF16)] + extra,
            grid=(2,) if cfg.get("dyn", False) else (),
            in_specs=[anyspec, anyspec, anyspec] + [vm] * 12,
            out_specs=[anyspec] * (1 + len(extra)),
            scratch_shapes=K.scratch(cfg),
            compiler_params=pltpu.CompilerParams(vmem_limit_bytes=cfg["vmem_mb"] * 1024 * 1024, flags=cfg.get("flags")),
        )(x, B_w1, B_w2, A_A_re, A_A_im, A_B_re, A_B_im, A_C_re, A_C_im,
          A_log_dt.reshape(NG, 128), A_Dskip.reshape(NG, 128), B_b1.reshape(F // 128, 128), B_b2.reshape(NG, 128),
          jnp.asarray(_MC), jnp.asarray(_GP))
        return out[0].reshape(1, L, D) if not extra else out
    return fn


@jax.jit
def pallas_parallel_sum__ssm_conv_s4__mixer_channel_mlp__prompt_kernel(
    A_u, A_A_re, A_A_im, A_B_re, A_B_im, A_C_re, A_C_im, A_log_dt, A_Dskip, B_x, B_w1, B_b1, B_w2, B_b2,
):
    return build()(A_u, A_A_re, A_A_im, A_B_re, A_B_im, A_C_re, A_C_im, A_log_dt, A_Dskip, B_x, B_w1, B_b1, B_w2, B_b2)
```

```python
import numpy as np
import jax
import jax.numpy as jnp
import jax.experimental.pallas as pl
import jax.experimental.pallas.tpu as pltpu

L, D, N, F = 2048, 512, 128, 1792
Q = 128
NB = L // Q
NG = D // 128
MT = 256
FC = 128
NT = L // MT
S = 132
BS = 136
PS = NB * BS + 8
VS = 136
PAD = 8
PC = 16
MB = 2
MAC_TIE = 2
LN_RC = 8
FIN_RC = 32
H2_SPLIT = 14
F32, BF16, I32 = jnp.float32, jnp.bfloat16, jnp.int32

WIN = dict(DU=(0.0, 0.06), P=(0.0, 0.14), MAC=(0.12, 0.78), KV=(0.145, 0.85), KD=(0.16, 0.865),
           ID=(0.905, 0.95), DK=(0.94, 0.995),
           DU3=(0.0, 0.06), MAC3=(0.16, 0.84), ID3=(0.95, 1.0), FINA=(0.0, 0.9))


def _np_bf16_bits(a):
    u = np.ascontiguousarray(a, dtype=np.float32).view(np.uint32).astype(np.uint64)
    return ((u + 0x7FFF + ((u >> 16) & 1)) >> 16).astype(np.uint32)


def _np_pack_rows(a):
    b = _np_bf16_bits(a)
    return (b[0::2] | (b[1::2] << 16)).view(np.int32)


def _bpos(b):
    return 16 * (b // 16) + 2 * (b % 8) + (b % 16) // 8


def _make_tables():
    lag = (_np_bf16_bits(np.arange(L, dtype=np.float32)) << 16).view(np.float32).astype(np.int64)
    k = np.concatenate([np.arange(0, Q, 2), np.arange(1, Q, 2)]).astype(np.float64)
    t = np.arange(Q, dtype=np.float64)
    th = 2.0 * np.pi * (k[:, None] + 0.5) * t[None, :] / (2 * Q)
    fwd = np.concatenate([np.cos(th), -np.sin(th)], 0)
    mats, cls = [fwd], []
    for i in range(NB):
        m = np.zeros((2 * Q, Q))
        for tt in range(Q):
            b = int(lag[Q * i + tt]) - Q * i
            assert 0 <= b <= Q
            if b == Q:
                assert i >= 2
                b = 1
            else:
                assert i < 2 or b != 1
            m[:, _bpos(b)] += fwd[:, tt]
        for c in range(1, len(mats)):
            if np.array_equal(mats[c], m):
                cls.append(c)
                break
        else:
            mats.append(m)
            cls.append(len(mats) - 1)
    thi = 2.0 * np.pi * (k[None, :] + 0.5) * t[:, None] / (2 * Q)
    inv = np.stack([np.cos(thi) / Q, -np.sin(thi) / Q], 2).reshape(Q, 2 * Q)
    return (np.stack([_np_pack_rows(m) for m in mats]),
            np.stack([_np_pack_rows(inv[:, :Q]), _np_pack_rows(inv[:, Q:])]), tuple(cls))


_MC, _GP, _CLS = _make_tables()
_ABSENT = 0x7FC17FC1
assert not (_MC == _ABSENT).any()


def _cmul(ar, ai, br, bi):
    return ar * br - ai * bi, ar * bi + ai * br


def _csq(ar, ai):
    t = ar * ai
    return ar * ar - ai * ai, t + t


def _nt(a, b):
    return jax.lax.dot_general(a, b, (((1,), (1,)), ((), ())), preferred_element_type=F32)


def _nn(a, b):
    return jnp.dot(a, b, preferred_element_type=F32)


def _pack(lo, hi):
    return pltpu.pack_elementwise([lo, hi], packed_dtype=BF16)


def _unpack(w):
    return (pltpu.unpack_elementwise(w, index=0, packed_dtype=BF16, unpacked_dtype=F32),
            pltpu.unpack_elementwise(w, index=1, packed_dtype=BF16, unpacked_dtype=F32))


def _bf(w):
    return pltpu.bitcast(w, BF16)


def _gelu2(x):
    c1 = 0.7978845608028654
    c2 = 0.7978845608028654 * 0.044715
    return x + x * jnp.tanh(x * (c1 + c2 * (x * x)))


def _rows(g, n):
    if isinstance(g, int):
        return pl.ds(g * n, n)
    return pl.ds(pl.multiple_of(g * n, 8), n)


def _run(gen):
    for _ in gen:
        pass


def _take(gen, w):
    t = 0.0
    while t < w - 1e-6:
        x = next(gen)
        t += x
        yield x


def _chain(*gens):
    for g in gens:
        yield from g


def _merge(*streams):
    st = [[g, 0.0, float(w), a, b] for g, w, a, b in streams]
    while st:
        s = min(st, key=lambda q: q[3] + (q[4] - q[3]) * q[1] / q[2])
        try:
            s[1] += next(s[0])
        except StopIteration:
            st.remove(s)


class _Emit:
    def __init__(self, refs):
        (self.x_hbm, self.w1_hbm, self.w2_hbm, self.p0, self.p1, self.p2, self.p3, self.p4, self.p5,
         self.ldt_h, self.dsk_h, self.b1_h, self.b2_h, self.mc_h, self.gp_h, self.out_hbm,
         self.are, self.aim, self.bre, self.bim, self.cre, self.cim, self.ldt, self.dsk, self.b1, self.b2,
         self.mc, self.gp, self.x_s, self.w1_s, self.w2_s, self.xn_s, self.dt_s, self.vbr, self.vbi,
         self.lar, self.lai, self.zz, self.xk, self.vs, self.ku, self.y_s, self.r_s, self.acc_s,
         self.st_s, self.o_s, self.sems, self.osems) = refs
        self.tokens = None
        self.t0 = self.now = 0.0
        self.total = 1.0
        self.tok_t0, self.tok_dur = 0.0, 1.0
        self.cps = []
        self.p_rows = self.kv_done = self.du_done = 0
        self.kd_done = 128
        self.mac_done = True

    def schedule(self, leads, others):
        ls = [[g, 0.0, float(c), a, b] for g, c, a, b in leads]
        vs = [[g, 0.0, float(w), a, b] for g, w, a, b in others]
        self.total = sum(s[2] for s in ls)
        self.tokens = None
        tau = 0.0

        def tm(s):
            return s[3] + (s[4] - s[3]) * s[1] / s[2]
        while ls or vs:
            if ls:
                s = min(ls, key=tm)
                self.t0 = self.now = tau
                try:
                    c = next(s[0])
                    s[1] += c
                    tau += c / self.total
                except StopIteration:
                    ls.remove(s)
                    continue
            while vs:
                o = min(vs, key=tm)
                if ls and tm(o) >= tau:
                    break
                self.now = tm(o)
                try:
                    o[1] += next(o[0])
                except StopIteration:
                    vs.remove(o)
        self.tokens = None

    def post(self, v, cycles):
        self.tokens = [v[r:r + 8, 0:128] for r in range(0, v.shape[0], 16)]
        self.tok_t0, self.tok_dur = self.t0, cycles / self.total

    def tie(self, *vals):
        if self.tokens is None:
            return vals
        frac = (self.now - self.tok_t0) / self.tok_dur
        tok = self.tokens[max(0, min(len(self.tokens) - 1, int(frac * len(self.tokens))))]
        keep = self.mc[0, 0:8, :] != _ABSENT
        out = []
        for v in vals:
            t = tok if v.dtype == F32 else jax.lax.bitcast_convert_type(tok, v.dtype)
            if v.shape != (8, 128):
                out.append(jnp.where(keep[None], v.reshape(-1, 8, 128), t[None]).reshape(v.shape))
            else:
                out.append(jnp.where(keep, v, t))
        return out

    def dt_columns(self):
        dt_row = jnp.exp(self.ldt[...].astype(F32)).astype(BF16).astype(F32)
        for g in range(NG):
            self.dt_s[pl.ds(g * 128, 128), :] = jnp.broadcast_to(dt_row[g:g + 1, :], (128, 128)).T

    def precompute(self, g):
        assert self.kd_done == 128
        self.p_rows = 0
        for c in range(128 // PC):
            if isinstance(g, int):
                src = pl.ds(g * 128 + c * PC, PC)
            else:
                src = pl.ds(pl.multiple_of(g * 128 + c * PC, 8), PC)
            dt, = self.tie(self.dt_s[src, :])

            def ld(ref):
                return ref[src, :].astype(F32)
            lr, li = dt * ld(self.are), dt * ld(self.aim)
            br, bi = dt * ld(self.bre), dt * ld(self.bim)
            cr, ci = ld(self.cre), ld(self.cim)
            a = (cr * br - ci * bi, -(cr * bi + ci * br))
            mag = jnp.exp(lr)
            z1 = (mag * jnp.cos(li), mag * jnp.sin(li))
            yield 3.0
            z2 = _csq(*z1)
            z3 = _cmul(*z2, *z1)
            z4 = _csq(*z2)
            pw = [(jnp.ones((PC, 128), F32), jnp.zeros((PC, 128), F32)), z1, z2, z3, z4,
                  _cmul(*z4, *z1), _csq(*z3), _cmul(*z4, *z3)]
            for b0 in range(8):
                self.vbr[pl.ds(b0 * S + c * PC, PC), :] = pw[b0][0]
                self.vbi[pl.ds(b0 * S + c * PC, PC), :] = pw[b0][1]
            z = z4
            for q in range(4):
                z = _csq(*z)
                self.zz[pl.ds((2 * q) * 128 + c * PC, PC), :] = z[0]
                self.zz[pl.ds((2 * q + 1) * 128 + c * PC, PC), :] = z[1]
            z = _csq(*z)
            yield 2.0
            zc = (z[0], -z[1])
            for i in range(NB):
                slab = (i // 2) + 8 * (i % 2)
                self.lar[pl.ds(slab * S + c * PC, PC), :] = a[0]
                self.lai[pl.ds(slab * S + c * PC, PC), :] = a[1]
                a = _cmul(*a, *zc)
                if i == 7:
                    yield 1.5
            self.xk[pl.ds((NB + 1) * S + c * PC, PC), :] = jnp.broadcast_to(
                jnp.sum(a[0], axis=1, keepdims=True), (PC, 128))
            self.p_rows = (c + 1) * PC
            yield 1.5

    def vandermonde(self, paced):
        self.kv_done = 0
        for d in range(128):
            assert self.p_rows > d

            def zrow(q):
                return (jnp.broadcast_to(self.zz[pl.ds((2 * q) * 128 + d, 1), :], (8, 128)),
                        jnp.broadcast_to(self.zz[pl.ds((2 * q + 1) * 128 + d, 1), :], (8, 128)))

            def put(j, a, b):
                self.vs[pl.ds(d * VS + 8 * j, 8), :] = _pack(a[0], b[0])
                self.vs[pl.ds(d * VS + 64 + 8 * j, 8), :] = _pack(a[1], b[1])
            v0 = (self.vbr[pl.ds(d, 8, stride=S), :], self.vbi[pl.ds(d, 8, stride=S), :])
            v1 = _cmul(*v0, *self.tie(*zrow(0)))
            if paced:
                z = zrow(1)
                for j in range(8):
                    if j > 0:
                        v0, v1 = _cmul(*v0, *z), _cmul(*v1, *z)
                    put(j, v0, v1)
            else:
                v = [v0, v1]
                for q in range(1, 4):
                    z = zrow(q)
                    v += [_cmul(*u, *z) for u in v]
                for j in range(8):
                    put(j, v[2 * j], v[2 * j + 1])
            self.kv_done = d + 1
            yield 1.0

    def kernel_taps(self):
        self.kd_done = 0
        self.xk[pl.ds(NB * S, 128), :] = self.xk[pl.ds((NB + 1) * S, 128), :]
        for d in range(128):
            assert self.kv_done > d

            def lhs(ref):
                return _bf(_pack(ref[pl.ds(d, 8, stride=S), :], ref[pl.ds(8 * S + d, 8, stride=S), :]))
            self.xk[pl.ds(d, NB, stride=S), :] = (
                _nt(lhs(self.lar), _bf(self.vs[pl.ds(d * VS, 64), :]))
                + _nt(lhs(self.lai), _bf(self.vs[pl.ds(d * VS + 64, 64), :])))
            self.kd_done = d + 1
            yield 1.0

    def dft_k(self):
        assert self.kd_done == 128 and self.mac_done
        lane = jax.lax.broadcasted_iota(I32, (128, 128), 1)
        prev = None
        for i in range(NB):
            xt = self.xk[pl.ds(i * S, 128), :]
            if i >= 2:
                nx = self.xk[pl.ds((i + 1) * S, 128), :]
                xt = jnp.where(lane == _bpos(1), pltpu.roll(nx, _bpos(1), 1), xt)
            kf = _nt(_bf(self.mc[_CLS[i]]), xt.astype(BF16))
            a, b = kf[:128], kf[128:]
            if prev is None:
                c, e = a, b
            else:
                pa, pb = prev
                c = jnp.concatenate([a[:64] - pb[:64], a[64:] + pb[64:]], axis=0)
                e = jnp.concatenate([b[:64] + pa[:64], b[64:] - pa[64:]], axis=0)
            prev = (a, b)
            self.ku[pl.ds(0 * PS + i * BS, 128), :] = c
            self.ku[pl.ds(1 * PS + i * BS, 128), :] = e - c
            self.ku[pl.ds(2 * PS + i * BS, 128), :] = e + c
            if i % 4 == 3:
                self.post(kf, 256)
                yield 256

    def dft_u(self, g):
        assert self.mac_done
        self.du_done = 0
        for j in range(NB):
            uf = _nn(_bf(self.mc[0]), _bf(self.xn_s[g, pl.ds(j * 64, 64), :]))
            a, b = uf[:128], uf[128:]
            self.ku[pl.ds(3 * PS + j * BS, 128), :] = a
            self.ku[pl.ds(4 * PS + j * BS, 128), :] = b
            self.ku[pl.ds(5 * PS + j * BS, 128), :] = a + b
            self.du_done = j + 1
            if j % 4 == 3:
                self.post(uf, 256)
                yield 256

    def block_conv(self):
        assert self.du_done == NB
        self.mac_done = False
        for v in range(16):
            def ld(q, blk):
                return self.ku[pl.ds(q * PS + blk * BS + 8 * v, 8), :]
            for m0 in range(0, NB, MB):
                ms = list(range(m0, m0 + MB))
                s1, s2, s3, us = {}, {}, {}, {}
                for i in range(ms[-1] + 1):
                    c, e, f = ld(0, i), ld(1, i), ld(2, i)
                    if i % MAC_TIE == 0:
                        c, e, f = self.tie(c, e, f)
                    n = 0
                    for m in ms:
                        j = m - i
                        if j < 0:
                            continue
                        if j not in us:
                            us[j] = (ld(3, j), ld(4, j), ld(5, j))
                        ua, ub, ug = us[j]
                        if m in s1:
                            s1[m], s2[m], s3[m] = s1[m] + c * ug, s2[m] + e * ua, s3[m] + f * ub
                        else:
                            s1[m], s2[m], s3[m] = c * ug, e * ua, f * ub
                        n += 1
                    yield n / 136.0
                for m in ms:
                    self.y_s[m, pl.ds(8 * v, 8), :] = _pack(s1[m] - s3[m], s1[m] + s2[m])
        self.mac_done = True

    def idft(self, g):
        assert self.mac_done
        for m in range(NB):
            gm = jnp.concatenate([_bf(self.gp[0]), _bf(self.gp[1])], axis=1)
            yo = _nn(gm, _bf(self.y_s[m, pl.ds(0, 128), :]))
            self.r_s[g, pl.ds(m * 128, 128), :] = yo
            if m % 4 == 3:
                self.post(yo, 256)
                yield 256

    def layernorm(self, n0, n1):
        inv = 1.0 / D

        def words(r):
            w = self.x_s[pl.ds(r * LN_RC, LN_RC), :]
            if self.tokens is not None:
                w = jnp.concatenate([self.tie(w[:, :128])[0], w[:, 128:]], axis=1)
            return _unpack(w)
        for r in range(n0, n1):
            for t, v in enumerate(words(r)):
                self.st_s[t, pl.ds(r * LN_RC, LN_RC), :] = jnp.broadcast_to(
                    jnp.sum(v, axis=1, keepdims=True) * inv, (LN_RC, 128))
            yield 0.2
        for r in range(n0, n1):
            for t, v in enumerate(words(r)):
                mu = self.st_s[t, pl.ds(r * LN_RC, LN_RC), :]
                sq = None
                for kk in range(NG):
                    c = v[:, kk * 128:(kk + 1) * 128] - mu
                    sq = c * c if sq is None else sq + c * c
                var = jnp.sum(sq, axis=1, keepdims=True) * inv
                self.st_s[2 + t, pl.ds(r * LN_RC, LN_RC), :] = jnp.broadcast_to(
                    jax.lax.rsqrt(var + 1e-5), (LN_RC, 128))
            yield 0.5
        for r in range(n0, n1):
            ev, od = words(r)
            mu = [self.st_s[t, pl.ds(r * LN_RC, LN_RC), :] for t in range(2)]
            rs = [self.st_s[2 + t, pl.ds(r * LN_RC, LN_RC), :] for t in range(2)]
            for kk in range(NG):
                sl = slice(kk * 128, (kk + 1) * 128)
                self.xn_s[kk, pl.ds(r * LN_RC, LN_RC), :] = _pack((ev[:, sl] - mu[0]) * rs[0],
                                                                  (od[:, sl] - mu[1]) * rs[1])
            yield 0.3

    def mlp(self, r):
        cyc = MT * FC // 128
        for c in range(F // FC):
            xt = jnp.concatenate([_bf(self.xn_s[kk, _rows(r, MT // 2), :]) for kk in range(NG)], axis=1)
            h = _nn(xt, _bf(self.w1_s[:, c * FC:(c + 1) * FC])) + self.b1[pl.ds(c, 1), :].astype(F32)
            self.post(h, cyc)
            yield cyc
            p = _nn(_gelu2(h).astype(BF16), _bf(self.w2_s[c * FC // 2:(c + 1) * FC // 2, :]))
            self.post(p, cyc)
            for g in range(NG):
                if c == 0:
                    self.acc_s[g, _rows(r, MT), :] = p[:, g * 128:(g + 1) * 128]
                else:
                    self.acc_s[g, _rows(r, MT), :] += p[:, g * 128:(g + 1) * 128]
            yield cyc

    def finalize(self, r, g0, g1):
        for t in range(MT // FIN_RC):
            r0 = r * MT + t * FIN_RC
            outs = []
            for g in range(g0, g1):
                a = self.acc_s[g, pl.ds(r0, FIN_RC), :]
                if g == g0:
                    a, = self.tie(a)
                y = self.r_s[g, pl.ds(r0, FIN_RC), :]
                xx = _bf(self.x_s[pl.ds(r0 // 2, FIN_RC // 2), g * 128:(g + 1) * 128]).astype(F32)
                xn = _bf(self.xn_s[g, pl.ds(r0 // 2, FIN_RC // 2), :]).astype(F32)
                dk = self.dsk[pl.ds(g, 1), :].astype(F32)
                bb = self.b2[pl.ds(g, 1), :].astype(F32)
                outs.append(xx + (y + xn * dk) + (0.5 * a + bb))
            self.o_s[pl.ds(r0, FIN_RC), g0 * 128:g1 * 128] = jnp.concatenate(outs, axis=1).astype(BF16)
            yield (g1 - g0) * FIN_RC / 256.0
        sl = (pl.ds(r * MT, MT), pl.ds(g0 * 128, (g1 - g0) * 128))
        cp = pltpu.make_async_copy(self.o_s.at[sl], self.out_hbm.at[sl], self.osems.at[len(self.cps)])
        cp.start()
        self.cps.append(cp)


def _kernel(*refs):
    k = _Emit(refs)
    srcs = (k.p0, k.p1, k.p2, k.p3, k.p4, k.p5)
    dsts = (k.are, k.aim, k.bre, k.bim, k.cre, k.cim)

    def copy(a, b, sem):
        return pltpu.make_async_copy(a, b, k.sems.at[sem])

    def params(r0, n, sem):
        return [copy(a.at[pl.ds(r0, n)], b.at[pl.ds(r0, n)], sem) for a, b in zip(srcs, dsts)]
    xw = k.x_hbm.bitcast(I32)
    cp_a = params(0, 128, 0) + [copy(k.ldt_h, k.ldt, 0)]
    cp_m = [copy(k.mc_h, k.mc, 1), copy(k.b1_h, k.b1, 1)]
    cp_w = [copy(xw.at[pl.ds(0, MT // 2)], k.x_s.at[pl.ds(0, MT // 2)], 2),
            copy(k.w1_hbm.bitcast(I32), k.w1_s, 3), copy(k.w2_hbm.bitcast(I32), k.w2_s, 4)]
    cp_x = copy(xw.at[pl.ds(MT // 2, (L - MT) // 2)], k.x_s.at[pl.ds(MT // 2, (L - MT) // 2)], 5)
    cp_c = params(128, D - 128, 6) + [copy(k.gp_h, k.gp, 6), copy(k.dsk_h, k.dsk, 6), copy(k.b2_h, k.b2, 6)]
    for cp in cp_a + cp_m + cp_w + [cp_x] + cp_c:
        cp.start()

    for cp in cp_a:
        cp.wait()
    k.dt_columns()
    _run(k.precompute(0))
    _merge((k.vandermonde(False), 128, 0.0, 1.0), (k.kernel_taps(), 128, 0.02, 1.02))
    for cp in cp_m:
        cp.wait()
    _run(k.dft_k())

    for cp in cp_w:
        cp.wait()
    n0, n1 = MT // 2 // LN_RC, L // 2 // LN_RC
    _run(k.layernorm(0, n0))
    dots = 2 * (F // FC)
    cyc = MT * FC // 128
    first = k.mlp(0)
    _run(_take(first, H2_SPLIT * cyc))
    cp_x.wait()
    k.schedule([(first, (dots - H2_SPLIT) * cyc, 0.0, 1.0)], [(k.layernorm(n0, n1), n1 - n0, 0.0, 0.97)])
    for cp in cp_c:
        cp.wait()

    def step(g, carry):
        k.schedule(
            [(_chain(k.mlp(2 * g + 1), k.mlp(2 * g + 2)), 2 * dots * cyc, 0.0, 1.0),
             (k.dft_u(g), 1024, *WIN["DU"]), (k.idft(g), 1024, *WIN["ID"]), (k.dft_k(), 1024, *WIN["DK"])],
            [(k.precompute(g + 1), 128 // PC * 8.0, *WIN["P"]), (k.block_conv(), 16, *WIN["MAC"]),
             (k.vandermonde(True), 128, *WIN["KV"]), (k.kernel_taps(), 128, *WIN["KD"])])
        return carry
    jax.lax.fori_loop(0, NG - 1, step, 0)

    g = NG - 1
    k.schedule(
        [(k.mlp(NT - 1), dots * cyc, 0.0, 1.0), (k.idft(g), 1024, *WIN["ID3"]), (k.dft_u(g), 1024, *WIN["DU3"])],
        [(k.block_conv(), 16, *WIN["MAC3"]),
         (_chain(*[k.finalize(r, 0, NG - 1) for r in range(NT - 1)]), (NT - 1) * 3.0, *WIN["FINA"])])
    _run(k.finalize(NT - 1, 0, NG))
    for r in range(NT - 1):
        _run(k.finalize(r, NG - 1, NG))
    for cp in k.cps:
        cp.wait()


def _scratch():
    vm = pltpu.VMEM
    return [vm((D, N), BF16)] * 6 + [
        vm((NG, 128), BF16), vm((NG, 128), BF16), vm((F // 128, 128), BF16), vm((NG, 128), BF16),
        vm(_MC.shape, I32), vm(_GP.shape, I32),
        vm((L // 2, D), I32), vm((D // 2, F), I32), vm((F // 2, D), I32),
        vm((NG, L // 2 + PAD, 128), I32),
        vm((D, 128), F32),
        vm((8 * S, 128), F32), vm((8 * S, 128), F32),
        vm((NB * S, 128), F32), vm((NB * S, 128), F32),
        vm((8 * 128, 128), F32),
        vm(((NB + 2) * S, 128), F32),
        vm((128 * VS, 128), I32),
        vm((6 * PS, 128), F32),
        vm((NB, 128 + PAD, 128), I32),
        vm((NG, L + PAD, 128), F32), vm((NG, L + PAD, 128), F32),
        vm((4, L // 2 + PAD, 128), F32),
        vm((L, D), BF16),
        pltpu.SemaphoreType.DMA((7,)), pltpu.SemaphoreType.DMA((2 * NT,)),
    ]


@jax.jit
def pallas_parallel_sum__ssm_conv_s4__mixer_channel_mlp__prompt_kernel(
    A_u: jax.Array,
    A_A_re: jax.Array,
    A_A_im: jax.Array,
    A_B_re: jax.Array,
    A_B_im: jax.Array,
    A_C_re: jax.Array,
    A_C_im: jax.Array,
    A_log_dt: jax.Array,
    A_Dskip: jax.Array,
    B_x: jax.Array,
    B_w1: jax.Array,
    B_b1: jax.Array,
    B_w2: jax.Array,
    B_b2: jax.Array,
):
    del B_x
    hbm = pl.BlockSpec(memory_space=pl.ANY)
    out = pl.pallas_call(
        _kernel,
        out_shape=jax.ShapeDtypeStruct((L, D), BF16),
        in_specs=[hbm] * 15,
        out_specs=hbm,
        scratch_shapes=_scratch(),
        compiler_params=pltpu.CompilerParams(vmem_limit_bytes=100 * 1024 * 1024),
    )(A_u.reshape(L, D), B_w1, B_w2, A_A_re, A_A_im, A_B_re, A_B_im, A_C_re, A_C_im,
      A_log_dt.reshape(NG, 128), A_Dskip.reshape(NG, 128), B_b1.reshape(F // 128, 128), B_b2.reshape(NG, 128),
      jnp.asarray(_MC), jnp.asarray(_GP))
    return out.reshape(1, L, D)
```
